```python
import os as _os
_os.environ.setdefault("JAX_PLATFORMS", "cpu")
import jax
import jax.numpy as jnp

def _softmax(x, axis=-1):
    return jax.nn.softmax(x, axis=axis)
def _gelu(x):
    return jax.nn.gelu(x, approximate=True)
def _silu(x):
    return jax.nn.silu(x)
def _sigmoid(x):
    return jax.nn.sigmoid(x)
def _layernorm(x, axis=-1, eps=1e-5):
    m = jnp.mean(x, axis=axis, keepdims=True)
    v = jnp.var(x, axis=axis, keepdims=True)
    return (x - m) / jnp.sqrt(v + eps)
def _scatter_add(tgt, idx, src, axis=0):
    return tgt.at[idx].add(src)
def _segment_sum(src, seg, n):
    return jax.ops.segment_sum(src, seg, n)
class _Rng:
    def __init__(self, key):
        self._k = key
    def _next(self):
        self._k, sub = jax.random.split(self._k)
        return sub
    def normal(self, shape):
        return jax.random.normal(self._next(), shape, dtype=jnp.bfloat16)
    def randint(self, lo, hi, shape):
        return jax.random.randint(self._next(), shape, lo, hi, dtype=jnp.int32)
    def uniform(self, shape, lo=0.0, hi=1.0):
        return jax.random.uniform(self._next(), shape, jnp.bfloat16, lo, hi)
    def permutation(self, n):
        return jax.random.permutation(self._next(), n)


kernel_name = 'parallel_sum__sliding_local_dilated__glu_gated_geglu__prompt'

def setup_inputs():
    _rng = _Rng(jax.random.key(int.from_bytes(__import__("os").urandom(4), "little")))
    _w = (lambda a: (lambda t: t.astype(jnp.bfloat16) if jnp.issubdtype(t.dtype, jnp.floating) else t)(jnp.asarray(a)))
    def _A_setup():
        B, S, D = 1, 2048, 512
        return {
            "x": _w((lambda *s: _rng.normal(s) * 0.05)(B, S, D)),
            "wqkv": _w((lambda *s: _rng.normal(s) * 0.05)(D, 3 * D)),
            "wo": _w((lambda *s: _rng.normal(s) * 0.05)(D, D)),
        }
    _A_in = _A_setup()

    def _B_setup():
        B, S, Dm, Df = 1, 2048, 512, 1376
        return {
            "x": _w((lambda *s: _rng.normal(s) * 0.05)(B, S, Dm)),
            "w_gate": _w((lambda *s: _rng.normal(s) * 0.1)(Dm, Df) * (Dm ** -0.5)),
            "w_up": _w((lambda *s: _rng.normal(s) * 0.1)(Dm, Df) * (Dm ** -0.5)),
            "w_down": _w((lambda *s: _rng.normal(s) * 0.1)(Df, Dm) * (Df ** -0.5)),
        }
    _B_in = _B_setup()

    return {
        "A_x": _A_in["x"],
        "A_wqkv": _A_in["wqkv"],
        "A_wo": _A_in["wo"],
        "B_x": _B_in["x"],
        "B_w_gate": _B_in["w_gate"],
        "B_w_up": _B_in["w_up"],
        "B_w_down": _B_in["w_down"],
    }

def reference(A_x, A_wqkv, A_wo, B_x, B_w_gate, B_w_up, B_w_down):
    def _A_ref(x, wqkv, wo):
        B, S, D = x.shape
        H = 32; Dh = D // H
        W, dil = 8, 2
        qkv = (lambda x, *d: x.transpose(*d))((x @ wqkv).reshape(B, S, 3, H, Dh), 2, 0, 3, 1, 4)
        q, k, v = qkv[0], qkv[1], qkv[2]
        scale = Dh ** -0.5
        pos = jnp.arange(S)
        off = jnp.arange(W) * dil
        idx = pos[:, None] - off[None, :]
        mask = idx >= 0
        idx_c = jnp.where(mask, idx, 0).reshape(-1)
        kg = k[:, :, idx_c, :].reshape(B, H, S, W, Dh)
        vg = v[:, :, idx_c, :].reshape(B, H, S, W, Dh)
        logits = jnp.einsum("bhsd,bhswd->bhsw", q, kg) * scale
        logits = jnp.where(mask[None, None, :, :], logits, -1e9)
        attn = _softmax(logits, axis=-1)
        o = jnp.einsum("bhsw,bhswd->bhsd", attn, vg)
        return (lambda x, *d: x.transpose(*d))(o, 0, 2, 1, 3).reshape(B, S, D) @ wo

    def _B_ref(x, w_gate, w_up, w_down):
        g = jnp.einsum("bsd,df->bsf", x, w_gate)
        u = jnp.einsum("bsd,df->bsf", x, w_up)
        h = _gelu(g) * u
        return jnp.einsum("bsf,fd->bsd", h, w_down)

    x = A_x
    xn = _layernorm(x, axis=-1)
    return x + _A_ref(xn, A_wqkv, A_wo) + _B_ref(xn, B_w_gate, B_w_up, B_w_down)
```

```python
import functools

import jax
import jax.numpy as jnp
from jax import lax
import jax.experimental.pallas as pl
import jax.experimental.pallas.tpu as pltpu

S, D, DF = 2048, 512, 1376
DFP = 1408
HALO = 16
WIN, DIL = 8, 2
LOG2E = 1.4426950408889634
QSCALE = 0.25 * LOG2E
MASKED = -1e9 * LOG2E
f32, bf16, i32 = jnp.float32, jnp.bfloat16, jnp.int32
NT_DIMS = (((1,), (1,)), ((), ()))

X_TILES = ((0, 256), (256, 256), (512, 512), (1024, 512), (1536, 512))
G0, G1 = 256, 512
M1, GC = 512, 256
PM = 256
R = 16
MWL = 128
RP = 32
N_SEM = len(X_TILES) + 8 + 3 + S // PM + PM // MWL


def _pk(x):
    return pltpu.bitcast(x.astype(bf16), i32)


def _upk(x):
    return pltpu.bitcast(x, bf16)


def _half(r):
    return r // 2 if isinstance(r, int) else pl.multiple_of(r // 2, 8)


def _layernorm(x):
    m = jnp.mean(x, axis=-1, keepdims=True)
    xc = x - m
    var = jnp.mean(xc * xc, axis=-1, keepdims=True)
    return xc * lax.rsqrt(var + 1e-5)


def _geglu(g, u):
    c1 = 0.7978845608028654
    c2 = 0.7978845608028654 * 0.044715
    t = jnp.tanh(g * (c1 + c2 * (g * g)))
    hg = 0.5 * g
    return (hg * t + hg) * u


def _permute_cols(src):
    rows = src.shape[0]
    lane = lax.broadcasted_iota(i32, (rows, 128), 1)
    dd = lane // 32
    hh = lane % 8
    c = (lane % 32) // 8
    outs = []
    for cp in range(4):
        idx = 16 * hh + 4 * cp + dd
        acc = None
        for cs in range(4):
            g = jnp.take_along_axis(src[:, cs * 128:(cs + 1) * 128], idx, axis=1)
            acc = g if acc is None else jnp.where(c == cs, g, acc)
        outs.append(acc)
    return outs


def _attn_block(q_ref, k_ref, v_ref, o_ref, r0, masked):
    kr = r0 + HALO
    qs = [q_ref[c, pl.ds(r0, R), :] for c in range(4)]
    logits = []
    for w in range(WIN):
        acc = None
        for c in range(4):
            t = qs[c] * k_ref[c, pl.ds(kr - DIL * w, R), :]
            acc = t if acc is None else acc + t
        acc = acc + pltpu.roll(acc, 64, 1)
        acc = acc + pltpu.roll(acc, 32, 1)
        if masked and w > 0:
            row = lax.broadcasted_iota(i32, acc.shape, 0) + r0
            acc = jnp.where(row < DIL * w, MASKED, acc)
        logits.append(acc)
    m = logits[0]
    for w in range(1, WIN):
        m = jnp.maximum(m, logits[w])
    e = [jnp.exp2(logits[w] - m) for w in range(WIN)]
    l = e[0]
    for w in range(1, WIN):
        l = l + e[w]
    inv = 1.0 / l
    for c in range(4):
        acc = None
        for w in range(WIN):
            t = e[w] * v_ref[c, pl.ds(kr - DIL * w, R), :]
            acc = t if acc is None else acc + t
        o_ref[pl.ds(_half(r0), R // 2), c * 128:(c + 1) * 128] = _pk(acc * inv)


def _interleave(a, b):
    ta = sum(c for c, _ in a)
    tb = sum(c for c, _ in b)
    ia = ib = ca = cb = 0
    while ia < len(a) or ib < len(b):
        if ib >= len(b) or (ia < len(a) and ca * tb <= cb * ta):
            c, f = a[ia]
            f()
            ca += c
            ia += 1
        else:
            c, f = b[ib]
            f()
            cb += c
            ib += 1


def _kernel(x_hbm, wqkv_hbm, wo_hbm, wg_hbm, wu_hbm, wd_hbm, out_hbm,
            x_v, xn_p, wg_v, wu_v, wd_v, wqkv_v, wqkv_p, wo_v, wo_p, h_p,
            q_s, k_s, v_s, o_p, out_v, acc_s, sems):
    n_sem = [0]

    def copy(src, dst):
        c = pltpu.make_async_copy(src, dst, sems.at[n_sem[0]])
        n_sem[0] += 1
        return c

    def w_copy(a, b):
        b = min(b, DF)
        return (copy(wg_hbm.at[pl.ds(a, b - a), :], wg_v.at[pl.ds(a, b - a), :]),
                copy(wu_hbm.at[pl.ds(a, b - a), :], wu_v.at[pl.ds(a, b - a), :]))

    def start(*cs):
        for c in cs:
            c.start()

    def wait(*cs):
        for c in cs:
            c.wait()

    zpad = jnp.zeros((DFP - DF, D), bf16)
    wg_v[pl.ds(DF, DFP - DF), :] = zpad
    wu_v[pl.ds(DF, DFP - DF), :] = zpad
    wd_v[pl.ds(DF, DFP - DF), :] = zpad

    h0 = G0 // 2
    x_cp = [copy(x_hbm.at[pl.ds(r0, n), :], x_v.at[pl.ds(r0, n), :]) for r0, n in X_TILES]
    w_a, w_b, w_c, w_d = w_copy(0, h0), w_copy(h0, G0), w_copy(G0, G1), w_copy(G1, DFP)
    wqkv_cp = copy(wqkv_hbm, wqkv_v)
    wd_cp = copy(wd_hbm, wd_v.at[pl.ds(0, DF), :])
    wo_cp = copy(wo_hbm, wo_v)
    out_sem0 = n_sem[0]
    start(x_cp[0], *w_a, *w_b, *x_cp[1:], *w_c, *w_d, wqkv_cp, wo_cp, wd_cp)

    k_s[:, pl.ds(0, HALO), :] = jnp.zeros((4, HALO, 128), f32)
    v_s[:, pl.ds(0, HALO), :] = jnp.zeros((4, HALO, 128), f32)

    def gate_up(r0, m, a, b):
        xn = _upk(xn_p[pl.ds(r0 // 2, m // 2), :])
        g = lax.dot_general(xn, wg_v[pl.ds(a, b - a), :], NT_DIMS, preferred_element_type=f32)
        u = lax.dot_general(xn, wu_v[pl.ds(a, b - a), :], NT_DIMS, preferred_element_type=f32)
        h_p[pl.ds(r0 // 2, m // 2), pl.ds(a, b - a)] = _pk(_geglu(g, u))

    def norm(i):
        r0, n = X_TILES[i]
        xn_p[pl.ds(r0 // 2, n // 2), :] = _pk(_layernorm(x_v[pl.ds(r0, n), :].astype(f32)))

    wait(x_cp[0])
    norm(0)
    wait(*w_a)
    gate_up(*X_TILES[0], 0, h0)
    wait(*w_b, x_cp[1])
    norm(1)
    gate_up(*X_TILES[0], h0, G0)
    wait(x_cp[2])
    gate_up(*X_TILES[1], 0, G0)
    norm(2)
    for i in range(3, len(X_TILES)):
        wait(x_cp[i])
        if i == len(X_TILES) - 1:
            wait(*w_c)
        gate_up(*X_TILES[i - 1], 0, G0)
        norm(i)
    gate_up(*X_TILES[-1], 0, G0)
    for r in range(S // M1):
        for a in range(G0, G1, GC):
            gate_up(r * M1, M1, a, min(a + GC, G1))

    def perm_wqkv(r0):
        for m in range(3):
            outs = _permute_cols(pltpu.bitcast(wqkv_v[pl.ds(r0, RP), m * 512:(m + 1) * 512], i32))
            for cp in range(4):
                wqkv_p[pl.ds(r0 // 2, RP // 2), m * 512 + cp * 128:m * 512 + (cp + 1) * 128] = outs[cp]

    def perm_wo(n0):
        outs = _permute_cols(pltpu.bitcast(wo_v[:, pl.ds(n0, 128)].T, i32))
        for cp in range(4):
            wo_p[pl.ds(n0 // 2, 64), cp * 128:(cp + 1) * 128] = outs[cp]

    def qkv_task(r0, m, c):
        def f():
            xn = _upk(xn_p[pl.ds(_half(r0), PM // 2), :])
            y = jnp.dot(xn, _upk(wqkv_p[:, m * 512 + c * 128:m * 512 + (c + 1) * 128]),
                        preferred_element_type=f32)
            if m == 0:
                q_s[c, pl.ds(r0, PM), :] = y * QSCALE
            elif m == 1:
                k_s[c, pl.ds(r0 + HALO, PM), :] = y
            else:
                v_s[c, pl.ds(r0 + HALO, PM), :] = y
        return (4, f)

    def qkv_tasks(r0):
        return [qkv_task(r0, m, c) for m in range(3) for c in range(4)]

    def attn_task(r0, masked):
        return (1, lambda: _attn_block(q_s, k_s, v_s, o_p, r0, masked))

    def down_task(r0, n):
        def f():
            rows, cols = pl.ds(r0, PM), pl.ds(n * 128, 128)
            acc = jnp.dot(_upk(h_p[pl.ds(_half(r0), PM // 2), :]), wd_v[:, cols], preferred_element_type=f32)
            acc_s[n, rows, :] = acc + x_v[rows, cols].astype(f32)
        return (11, f)

    def out_proj(r0, m, n):
        rows, cols = pl.ds(r0, m), pl.ds(n * 128, 128)
        acc = lax.dot_general(_upk(o_p[pl.ds(_half(r0), m // 2), :]), _upk(wo_p[pl.ds(n * 64, 64), :]),
                              NT_DIMS, preferred_element_type=f32)
        out_v[rows, cols] = (acc + acc_s[n, rows, :]).astype(bf16)

    def out_copy(r0, m, sem):
        rows = pl.ds(r0, m)
        return pltpu.make_async_copy(out_v.at[rows, :], out_hbm.at[rows, :], sems.at[out_sem0 + sem])

    wait(*w_d, wqkv_cp, wo_cp, wd_cp)
    prep = ([(1, functools.partial(perm_wqkv, t * RP)) for t in range(D // RP)]
            + [(1, functools.partial(perm_wo, t * 128)) for t in range(4)])
    gu = [(1, functools.partial(gate_up, r * M1, M1, a, min(a + GC, DFP)))
          for r in range(S // M1) for a in range(G1, DFP, GC)]
    n_last = len(gu) // (S // M1)
    _interleave(gu[:-n_last], prep)
    for _, f in gu[-n_last:] + qkv_tasks(0):
        f()

    n_tiles = S // PM

    def step(t, last):
        dyn = not isinstance(t, int)
        r = pl.multiple_of(t * PM, PM) if dyn else t * PM
        mxu = [] if last else qkv_tasks(pl.multiple_of(r + PM, PM) if dyn else r + PM)
        mxu += [down_task(r, n) for n in range(4)]
        vpu = [attn_task(r + b * R, (not dyn) and t == 0 and b * R < DIL * WIN) for b in range(PM // R)]
        _interleave(mxu, vpu)
        m = MWL if last else PM
        for i in range(PM // m):
            for n in range(4):
                out_proj(r + i * m, m, n)
            out_copy(r + i * m, m, t + i).start()

    step(0, False)

    def body(t, carry):
        step(t, False)
        return carry

    lax.fori_loop(1, n_tiles - 1, body, 0)
    step(n_tiles - 1, True)

    for t in range(n_tiles - 1):
        out_copy(t * PM, PM, t).wait()
    for i in range(PM // MWL):
        out_copy((n_tiles - 1) * PM + i * MWL, MWL, n_tiles - 1 + i).wait()


@jax.jit
def pallas_parallel_sum__sliding_local_dilated__glu_gated_geglu__prompt_kernel(
    A_x: jax.Array,
    A_wqkv: jax.Array,
    A_wo: jax.Array,
    B_x: jax.Array,
    B_w_gate: jax.Array,
    B_w_up: jax.Array,
    B_w_down: jax.Array,
):
    del B_x
    hbm = pl.BlockSpec(memory_space=pltpu.HBM)
    out = pl.pallas_call(
        _kernel,
        in_specs=[hbm] * 6,
        out_specs=hbm,
        out_shape=jax.ShapeDtypeStruct((S, D), A_x.dtype),
        scratch_shapes=[
            pltpu.VMEM((S, D), bf16),
            pltpu.VMEM((S // 2, D), i32),
            pltpu.VMEM((DFP, D), bf16),
            pltpu.VMEM((DFP, D), bf16),
            pltpu.VMEM((DFP, D), bf16),
            pltpu.VMEM((D, 3 * D), bf16),
            pltpu.VMEM((D // 2, 3 * D), i32),
            pltpu.VMEM((D, D), bf16),
            pltpu.VMEM((D // 2, D), i32),
            pltpu.VMEM((S // 2, DFP), i32),
            pltpu.VMEM((4, S, 128), f32),
            pltpu.VMEM((4, S + HALO, 128), f32),
            pltpu.VMEM((4, S + HALO, 128), f32),
            pltpu.VMEM((S // 2, D), i32),
            pltpu.VMEM((S, D), bf16),
            pltpu.VMEM((4, S, 128), f32),
            pltpu.SemaphoreType.DMA((N_SEM,)),
        ],
        compiler_params=pltpu.CompilerParams(
            vmem_limit_bytes=110 * 1024 * 1024,
            flags={"XLA_TPU_EVENLY_DISTRIBUTE_CRITICAL_NODES": True},
        ),
    )(A_x.reshape(S, D), A_wqkv, A_wo, B_w_gate.T, B_w_up.T, B_w_down)
    return out.reshape(1, S, D)
```

```python
import functools

import jax
import jax.numpy as jnp
from jax import lax
import jax.experimental.pallas as pl
import jax.experimental.pallas.tpu as pltpu

S, D, DF = 2048, 512, 1376
DFM = 1280
DFP = 1408
HALO = 16
WIN, DIL = 8, 2
LOG2E = 1.4426950408889634
QSCALE = 0.25 * LOG2E
MASKED = -1e9 * LOG2E
f32, bf16, i32 = jnp.float32, jnp.bfloat16, jnp.int32
NT_DIMS = (((1,), (1,)), ((), ()))

X_TILES = ((0, 256), (256, 256), (512, 512), (1024, 512), (1536, 512))
G0, G1 = 256, 512
M1, GC = 512, 256
PM = 256
R = 16
MWL = 64
PEEL = 0
CHAIN = 0
TOK = 'r1'
UNROLL = 1
RP = 32
N_SEM = len(X_TILES) + 8 + 3 + S // PM + PM // MWL


def _pk(x):
    return pltpu.bitcast(x.astype(bf16), i32)


def _upk(x):
    return pltpu.bitcast(x, bf16)


def _half(r):
    return r // 2 if isinstance(r, int) else pl.multiple_of(r // 2, 8)


def _layernorm(x):
    m = jnp.mean(x, axis=-1, keepdims=True)
    xc = x - m
    var = jnp.mean(xc * xc, axis=-1, keepdims=True)
    return xc * lax.rsqrt(var + 1e-5)


def _geglu(g, u):
    c1 = 0.7978845608028654
    c2 = 0.7978845608028654 * 0.044715
    t = jnp.tanh(g * (c1 + c2 * (g * g)))
    hg = 0.5 * g
    return (hg * t + hg) * u


def _permute_cols(src):
    rows = src.shape[0]
    lane = lax.broadcasted_iota(i32, (rows, 128), 1)
    dd = lane // 32
    hh = lane % 8
    c = (lane % 32) // 8
    outs = []
    for cp in range(4):
        idx = 16 * hh + 4 * cp + dd
        acc = None
        for cs in range(4):
            g = jnp.take_along_axis(src[:, cs * 128:(cs + 1) * 128], idx, axis=1)
            acc = g if acc is None else jnp.where(c == cs, g, acc)
        outs.append(acc)
    return outs


def _attn_block(q_ref, k_ref, v_ref, o_ref, r0, masked, gate=None):
    kr = r0 + HALO
    qs = [q_ref[c, pl.ds(r0, R), :] for c in range(4)]
    if gate is not None:
        qs = [jnp.where(gate[0], gate[1], q) for q in qs]
    toks = {}
    logits = []
    for w in range(WIN):
        acc = None
        for c in range(4):
            t = qs[c] * k_ref[c, pl.ds(kr - DIL * w, R), :]
            acc = t if acc is None else acc + t
        toks['p'] = acc
        acc = acc + pltpu.roll(acc, 64, 1)
        toks['r1'] = acc
        acc = acc + pltpu.roll(acc, 32, 1)
        if masked and w > 0:
            row = lax.broadcasted_iota(i32, acc.shape, 0) + r0
            acc = jnp.where(row < DIL * w, MASKED, acc)
        logits.append(acc)
    m = logits[0]
    for w in range(1, WIN):
        m = jnp.maximum(m, logits[w])
    toks['m'] = m
    e = [jnp.exp2(logits[w] - m) for w in range(WIN)]
    l = e[0]
    for w in range(1, WIN):
        l = l + e[w]
    r = pl.reciprocal(l, approx=True)
    inv = r * (2.0 - l * r)
    for c in range(4):
        acc = None
        for w in range(WIN):
            t = e[w] * v_ref[c, pl.ds(kr - DIL * w, R), :]
            acc = t if acc is None else acc + t
        o_ref[pl.ds(_half(r0), R // 2), c * 128:(c + 1) * 128] = _pk(acc * inv)
        toks['o'] = acc
    return toks[TOK]


def _interleave(a, b):
    ta = sum(c for c, _ in a)
    tb = sum(c for c, _ in b)
    ia = ib = ca = cb = 0
    while ia < len(a) or ib < len(b):
        if ib >= len(b) or (ia < len(a) and ca * tb <= cb * ta):
            c, f = a[ia]
            f()
            ca += c
            ia += 1
        else:
            c, f = b[ib]
            f()
            cb += c
            ib += 1


def _kernel(x_hbm, wqkv_hbm, wo_hbm, wg_hbm, wu_hbm, wd_hbm, out_hbm,
            x_v, xn_p, wg_v, wu_v, wd_v, wqkv_v, wqkv_p, wo_v, wo_p, h_p,
            q_s, k_s, v_s, o_p, out_v, acc_s, sems):
    n_sem = [0]

    def copy(src, dst):
        c = pltpu.make_async_copy(src, dst, sems.at[n_sem[0]])
        n_sem[0] += 1
        return c

    def w_copy(a, b):
        b = min(b, DF)
        return (copy(wg_hbm.at[pl.ds(a, b - a), :], wg_v.at[pl.ds(a, b - a), :]),
                copy(wu_hbm.at[pl.ds(a, b - a), :], wu_v.at[pl.ds(a, b - a), :]))

    def start(*cs):
        for c in cs:
            c.start()

    def wait(*cs):
        for c in cs:
            c.wait()

    zpad = jnp.zeros((DFP - DF, D), bf16)
    wd_v[pl.ds(DF, DFP - DF), :] = zpad

    h0 = G0 // 2
    x_cp = [copy(x_hbm.at[pl.ds(r0, n), :], x_v.at[pl.ds(r0, n), :]) for r0, n in X_TILES]
    w_a, w_b, w_c, w_d = w_copy(0, h0), w_copy(h0, G0), w_copy(G0, G1), w_copy(G1, DFP)
    wqkv_cp = copy(wqkv_hbm, wqkv_v)
    wd_cp = copy(wd_hbm, wd_v.at[pl.ds(0, DF), :])
    wo_cp = copy(wo_hbm, wo_v)
    out_sem0 = n_sem[0]
    start(x_cp[0], *w_a, *w_b, *x_cp[1:], *w_c, *w_d, wqkv_cp, wo_cp, wd_cp)

    k_s[:, pl.ds(0, HALO), :] = jnp.zeros((4, HALO, 128), f32)
    v_s[:, pl.ds(0, HALO), :] = jnp.zeros((4, HALO, 128), f32)

    def gate_up(r0, m, a, b):
        xn = _upk(xn_p[pl.ds(r0 // 2, m // 2), :])
        g = lax.dot_general(xn, wg_v[pl.ds(a, b - a), :], NT_DIMS, preferred_element_type=f32)
        u = lax.dot_general(xn, wu_v[pl.ds(a, b - a), :], NT_DIMS, preferred_element_type=f32)
        h_p[pl.ds(r0 // 2, m // 2), pl.ds(a, b - a)] = _pk(_geglu(g, u))

    def gate_up_tail(r0, m):
        xn = _upk(xn_p[pl.ds(r0 // 2, m // 2), :])
        w = jnp.concatenate([wg_v[pl.ds(DFM, DF - DFM), :], wu_v[pl.ds(DFM, DF - DFM), :]], axis=0)
        gu_t = lax.dot_general(w, xn, NT_DIMS, preferred_element_type=f32)
        h_t = _geglu(gu_t[:DF - DFM], gu_t[DF - DFM:])
        h_t = jnp.concatenate([h_t, jnp.zeros((DFP - DF, m), f32)], axis=0)
        h_p[pl.ds(r0 // 2, m // 2), pl.ds(DFM, DFP - DFM)] = _pk(h_t.T)

    def norm(i):
        r0, n = X_TILES[i]
        xn_p[pl.ds(r0 // 2, n // 2), :] = _pk(_layernorm(x_v[pl.ds(r0, n), :].astype(f32)))

    wait(x_cp[0])
    norm(0)
    wait(*w_a)
    gate_up(*X_TILES[0], 0, h0)
    wait(*w_b, x_cp[1])
    norm(1)
    gate_up(*X_TILES[0], h0, G0)
    wait(x_cp[2])
    gate_up(*X_TILES[1], 0, G0)
    norm(2)
    for i in range(3, len(X_TILES)):
        wait(x_cp[i])
        if i == len(X_TILES) - 1:
            wait(*w_c)
        gate_up(*X_TILES[i - 1], 0, G0)
        norm(i)
    gate_up(*X_TILES[-1], 0, G0)
    for r in range(S // M1):
        for a in range(G0, G1, GC):
            gate_up(r * M1, M1, a, min(a + GC, G1))

    def perm_wqkv(r0):
        for m in range(3):
            outs = _permute_cols(pltpu.bitcast(wqkv_v[pl.ds(r0, RP), m * 512:(m + 1) * 512], i32))
            for cp in range(4):
                wqkv_p[pl.ds(r0 // 2, RP // 2), m * 512 + cp * 128:m * 512 + (cp + 1) * 128] = outs[cp]

    def perm_wo(n0):
        outs = _permute_cols(pltpu.bitcast(wo_v[:, pl.ds(n0, 128)].T, i32))
        for cp in range(4):
            wo_p[pl.ds(n0 // 2, 64), cp * 128:(cp + 1) * 128] = outs[cp]

    def qkv_task(r0, m, c):
        def f():
            xn = _upk(xn_p[pl.ds(_half(r0), PM // 2), :])
            y = jnp.dot(xn, _upk(wqkv_p[:, m * 512 + c * 128:m * 512 + (c + 1) * 128]),
                        preferred_element_type=f32)
            if m == 0:
                q_s[c, pl.ds(r0, PM), :] = y * QSCALE
            elif m == 1:
                k_s[c, pl.ds(r0 + HALO, PM), :] = y
            else:
                v_s[c, pl.ds(r0 + HALO, PM), :] = y
        return (4, f)

    def qkv_tasks(r0):
        return [qkv_task(r0, m, c) for m in range(3) for c in range(4)]

    def attn_task(r0, masked, st, b):
        def f():
            gate = (st['never'], st[b - CHAIN]) if CHAIN and b >= CHAIN else None
            st[b] = _attn_block(q_s, k_s, v_s, o_p, r0, masked, gate)
        return (1, f)

    def down_task(r0, n):
        def f():
            rows, cols = pl.ds(r0, PM), pl.ds(n * 128, 128)
            acc = jnp.dot(_upk(h_p[pl.ds(_half(r0), PM // 2), :]), wd_v[:, cols], preferred_element_type=f32)
            acc_s[n, rows, :] = acc + x_v[rows, cols].astype(f32)
        return (11, f)

    def out_proj(r0, m, n):
        rows, cols = pl.ds(r0, m), pl.ds(n * 128, 128)
        acc = lax.dot_general(_upk(o_p[pl.ds(_half(r0), m // 2), :]), _upk(wo_p[pl.ds(n * 64, 64), :]),
                              NT_DIMS, preferred_element_type=f32)
        out_v[rows, cols] = (acc + acc_s[n, rows, :]).astype(bf16)

    def out_copy(r0, m, sem):
        rows = pl.ds(r0, m)
        return pltpu.make_async_copy(out_v.at[rows, :], out_hbm.at[rows, :], sems.at[out_sem0 + sem])

    wait(*w_d, wqkv_cp, wo_cp, wd_cp)
    prep = ([(1, functools.partial(perm_wqkv, t * RP)) for t in range(D // RP)]
            + [(1, functools.partial(perm_wo, t * 128)) for t in range(4)])
    gu = []
    for r in range(S // M1):
        gu += [(min(a + GC, DFM) - a, functools.partial(gate_up, r * M1, M1, a, min(a + GC, DFM)))
               for a in range(G1, DFM, GC)]
        gu += [(DF - DFM, functools.partial(gate_up_tail, r * M1, M1))]
    n_last = len(gu) // (S // M1)
    _interleave(gu[:-n_last], prep)
    for _, f in gu[-n_last:] + qkv_tasks(0):
        f()

    n_tiles = S // PM

    def step(t, last):
        dyn = not isinstance(t, int)
        r = pl.multiple_of(t * PM, PM) if dyn else t * PM
        mxu = [] if last else qkv_tasks(pl.multiple_of(r + PM, PM) if dyn else r + PM)
        mxu += [down_task(r, n) for n in range(4)]
        st = {'never': k_s[0, pl.ds(0, R), :] != 0.0} if CHAIN else {}
        vpu = [attn_task(r + b * R, dyn and b * R < DIL * WIN, st, b) for b in range(PM // R)]
        _interleave(mxu, vpu)
        m = MWL if last else PM
        for i in range(PM // m):
            for n in range(4):
                out_proj(r + i * m, m, n)
            out_copy(r + i * m, m, t + i).start()

    def body(t, carry):
        for u in range(UNROLL):
            step(t * UNROLL + u, False)
        return carry

    lax.fori_loop(0, (n_tiles - 1 - PEEL) // UNROLL, body, 0)
    for t in range(n_tiles - 1 - PEEL, n_tiles - 1):
        step(t, False)
    step(n_tiles - 1, True)

    for t in range(n_tiles - 1):
        out_copy(t * PM, PM, t).wait()
    for i in range(PM // MWL):
        out_copy((n_tiles - 1) * PM + i * MWL, MWL, n_tiles - 1 + i).wait()


@jax.jit
def pallas_parallel_sum__sliding_local_dilated__glu_gated_geglu__prompt_kernel(
    A_x: jax.Array,
    A_wqkv: jax.Array,
    A_wo: jax.Array,
    B_x: jax.Array,
    B_w_gate: jax.Array,
    B_w_up: jax.Array,
    B_w_down: jax.Array,
):
    del B_x
    hbm = pl.BlockSpec(memory_space=pltpu.HBM)
    out = pl.pallas_call(
        _kernel,
        in_specs=[hbm] * 6,
        out_specs=hbm,
        out_shape=jax.ShapeDtypeStruct((S, D), A_x.dtype),
        scratch_shapes=[
            pltpu.VMEM((S, D), bf16),
            pltpu.VMEM((S // 2, D), i32),
            pltpu.VMEM((DF, D), bf16),
            pltpu.VMEM((DF, D), bf16),
            pltpu.VMEM((DFP, D), bf16),
            pltpu.VMEM((D, 3 * D), bf16),
            pltpu.VMEM((D // 2, 3 * D), i32),
            pltpu.VMEM((D, D), bf16),
            pltpu.VMEM((D // 2, D), i32),
            pltpu.VMEM((S // 2, DFP), i32),
            pltpu.VMEM((4, S, 128), f32),
            pltpu.VMEM((4, S + HALO, 128), f32),
            pltpu.VMEM((4, S + HALO, 128), f32),
            pltpu.VMEM((S // 2, D), i32),
            pltpu.VMEM((S, D), bf16),
            pltpu.VMEM((4, S, 128), f32),
            pltpu.SemaphoreType.DMA((N_SEM,)),
        ],
        compiler_params=pltpu.CompilerParams(
            vmem_limit_bytes=110 * 1024 * 1024,
            flags={"XLA_TPU_EVENLY_DISTRIBUTE_CRITICAL_NODES": True},
        ),
    )(A_x.reshape(S, D), A_wqkv, A_wo, B_w_gate.T, B_w_up.T, B_w_down)
    return out.reshape(1, S, D)
```

```python
import functools

import jax
import jax.numpy as jnp
from jax import lax
import jax.experimental.pallas as pl
import jax.experimental.pallas.tpu as pltpu

S, D, DF = 2048, 512, 1376
DFM = 1280
DFP = 1408
HALO = 16
WIN, DIL = 8, 2
LOG2E = 1.4426950408889634
QSCALE = 0.25 * LOG2E
MASKED = -1e9 * LOG2E
f32, bf16, i32 = jnp.float32, jnp.bfloat16, jnp.int32
NT_DIMS = (((1,), (1,)), ((), ()))

X_TILES = ((0, 256), (256, 256), (512, 512), (1024, 512), (1536, 512))
G0, G1 = 256, 512
M1, GC = 512, 256
PM = 256
R = 16
MWL = 64
FLAGS = {"XLA_TPU_EVENLY_DISTRIBUTE_CRITICAL_NODES": True}
RP = 32
N_SEM = len(X_TILES) + 8 + 3 + S // PM + PM // MWL


def _pk(x):
    return pltpu.bitcast(x.astype(bf16), i32)


def _upk(x):
    return pltpu.bitcast(x, bf16)


def _half(r):
    return r // 2 if isinstance(r, int) else pl.multiple_of(r // 2, 8)


def _layernorm(x):
    m = jnp.mean(x, axis=-1, keepdims=True)
    xc = x - m
    var = jnp.mean(xc * xc, axis=-1, keepdims=True)
    return xc * lax.rsqrt(var + 1e-5)


def _geglu(g, u):
    c1 = 0.7978845608028654
    c2 = 0.7978845608028654 * 0.044715
    t = jnp.tanh(g * (c1 + c2 * (g * g)))
    hg = 0.5 * g
    return (hg * t + hg) * u


def _permute_cols(src):
    rows = src.shape[0]
    lane = lax.broadcasted_iota(i32, (rows, 128), 1)
    dd = lane // 32
    hh = lane % 8
    c = (lane % 32) // 8
    outs = []
    for cp in range(4):
        idx = 16 * hh + 4 * cp + dd
        acc = None
        for cs in range(4):
            g = jnp.take_along_axis(src[:, cs * 128:(cs + 1) * 128], idx, axis=1)
            acc = g if acc is None else jnp.where(c == cs, g, acc)
        outs.append(acc)
    return outs


def _attn_block(q_ref, k_ref, v_ref, o_ref, r0, masked):
    kr = r0 + HALO
    qs = [q_ref[c, pl.ds(r0, R), :] for c in range(4)]
    logits = []
    for w in range(WIN):
        acc = None
        for c in range(4):
            t = qs[c] * k_ref[c, pl.ds(kr - DIL * w, R), :]
            acc = t if acc is None else acc + t
        acc = acc + pltpu.roll(acc, 64, 1)
        acc = acc + pltpu.roll(acc, 32, 1)
        if masked and w > 0:
            row = lax.broadcasted_iota(i32, acc.shape, 0) + r0
            acc = jnp.where(row < DIL * w, MASKED, acc)
        logits.append(acc)
    m = logits[0]
    for w in range(1, WIN):
        m = jnp.maximum(m, logits[w])
    e = [jnp.exp2(logits[w] - m) for w in range(WIN)]
    l = e[0]
    for w in range(1, WIN):
        l = l + e[w]
    r = pl.reciprocal(l, approx=True)
    inv = r * (2.0 - l * r)
    for c in range(4):
        acc = None
        for w in range(WIN):
            t = e[w] * v_ref[c, pl.ds(kr - DIL * w, R), :]
            acc = t if acc is None else acc + t
        o_ref[pl.ds(_half(r0), R // 2), c * 128:(c + 1) * 128] = _pk(acc * inv)


def _interleave(a, b):
    ta = sum(c for c, _ in a)
    tb = sum(c for c, _ in b)
    ia = ib = ca = cb = 0
    while ia < len(a) or ib < len(b):
        if ib >= len(b) or (ia < len(a) and ca * tb <= cb * ta):
            c, f = a[ia]
            f()
            ca += c
            ia += 1
        else:
            c, f = b[ib]
            f()
            cb += c
            ib += 1


def _kernel(x_hbm, wqkv_hbm, wo_hbm, wg_hbm, wu_hbm, wd_hbm, out_hbm,
            x_v, xn_p, wg_v, wu_v, wd_v, wqkv_v, wqkv_p, wo_v, wo_p, h_p,
            q_s, k_s, v_s, o_p, out_v, acc_s, sems):
    n_sem = [0]

    def copy(src, dst):
        c = pltpu.make_async_copy(src, dst, sems.at[n_sem[0]])
        n_sem[0] += 1
        return c

    def w_copy(a, b):
        b = min(b, DF)
        return (copy(wg_hbm.at[pl.ds(a, b - a), :], wg_v.at[pl.ds(a, b - a), :]),
                copy(wu_hbm.at[pl.ds(a, b - a), :], wu_v.at[pl.ds(a, b - a), :]))

    def start(*cs):
        for c in cs:
            c.start()

    def wait(*cs):
        for c in cs:
            c.wait()

    zpad = jnp.zeros((DFP - DF, D), bf16)
    wd_v[pl.ds(DF, DFP - DF), :] = zpad

    h0 = G0 // 2
    x_cp = [copy(x_hbm.at[pl.ds(r0, n), :], x_v.at[pl.ds(r0, n), :]) for r0, n in X_TILES]
    w_a, w_b, w_c, w_d = w_copy(0, h0), w_copy(h0, G0), w_copy(G0, G1), w_copy(G1, DFP)
    wqkv_cp = copy(wqkv_hbm, wqkv_v)
    wd_cp = copy(wd_hbm, wd_v.at[pl.ds(0, DF), :])
    wo_cp = copy(wo_hbm, wo_v)
    out_sem0 = n_sem[0]
    start(x_cp[0], *w_a, *w_b, *x_cp[1:], *w_c, *w_d, wqkv_cp, wo_cp, wd_cp)

    k_s[:, pl.ds(0, HALO), :] = jnp.zeros((4, HALO, 128), f32)
    v_s[:, pl.ds(0, HALO), :] = jnp.zeros((4, HALO, 128), f32)

    def gate_up(r0, m, a, b):
        xn = _upk(xn_p[pl.ds(r0 // 2, m // 2), :])
        g = lax.dot_general(xn, wg_v[pl.ds(a, b - a), :], NT_DIMS, preferred_element_type=f32)
        u = lax.dot_general(xn, wu_v[pl.ds(a, b - a), :], NT_DIMS, preferred_element_type=f32)
        h_p[pl.ds(r0 // 2, m // 2), pl.ds(a, b - a)] = _pk(_geglu(g, u))

    def gate_up_tail(r0, m):
        xn = _upk(xn_p[pl.ds(r0 // 2, m // 2), :])
        w = jnp.concatenate([wg_v[pl.ds(DFM, DF - DFM), :], wu_v[pl.ds(DFM, DF - DFM), :]], axis=0)
        gu_t = lax.dot_general(w, xn, NT_DIMS, preferred_element_type=f32)
        h_t = _geglu(gu_t[:DF - DFM], gu_t[DF - DFM:])
        h_t = jnp.concatenate([h_t, jnp.zeros((DFP - DF, m), f32)], axis=0)
        h_p[pl.ds(r0 // 2, m // 2), pl.ds(DFM, DFP - DFM)] = _pk(h_t.T)

    def norm(i):
        r0, n = X_TILES[i]
        xn_p[pl.ds(r0 // 2, n // 2), :] = _pk(_layernorm(x_v[pl.ds(r0, n), :].astype(f32)))

    wait(x_cp[0])
    norm(0)
    wait(*w_a)
    gate_up(*X_TILES[0], 0, h0)
    wait(*w_b, x_cp[1])
    norm(1)
    gate_up(*X_TILES[0], h0, G0)
    wait(x_cp[2])
    gate_up(*X_TILES[1], 0, G0)
    norm(2)
    gate_up(*X_TILES[2], 0, G0)
    wait(x_cp[3], x_cp[4], *w_c)
    gate_up(0, M1, G0, G1)
    norm(3)
    gate_up(M1, M1, G0, G1)
    norm(4)
    gate_up(*X_TILES[3], 0, G0)
    gate_up(*X_TILES[4], 0, G0)
    gate_up(2 * M1, M1, G0, G1)
    gate_up(3 * M1, M1, G0, G1)

    def perm_wqkv(r0):
        for m in range(3):
            outs = _permute_cols(pltpu.bitcast(wqkv_v[pl.ds(r0, RP), m * 512:(m + 1) * 512], i32))
            for cp in range(4):
                wqkv_p[pl.ds(r0 // 2, RP // 2), m * 512 + cp * 128:m * 512 + (cp + 1) * 128] = outs[cp]

    def perm_wo(n0):
        outs = _permute_cols(pltpu.bitcast(wo_v[:, pl.ds(n0, 128)].T, i32))
        for cp in range(4):
            wo_p[pl.ds(n0 // 2, 64), cp * 128:(cp + 1) * 128] = outs[cp]

    def qkv_task(r0, m, c):
        def f():
            xn = _upk(xn_p[pl.ds(_half(r0), PM // 2), :])
            y = jnp.dot(xn, _upk(wqkv_p[:, m * 512 + c * 128:m * 512 + (c + 1) * 128]),
                        preferred_element_type=f32)
            if m == 0:
                q_s[c, pl.ds(r0, PM), :] = y * QSCALE
            elif m == 1:
                k_s[c, pl.ds(r0 + HALO, PM), :] = y
            else:
                v_s[c, pl.ds(r0 + HALO, PM), :] = y
        return (4, f)

    def qkv_tasks(r0):
        return [qkv_task(r0, m, c) for m in range(3) for c in range(4)]

    def attn_task(r0, masked):
        return (1, lambda: _attn_block(q_s, k_s, v_s, o_p, r0, masked))

    def down_task(r0, n):
        def f():
            rows, cols = pl.ds(r0, PM), pl.ds(n * 128, 128)
            acc = jnp.dot(_upk(h_p[pl.ds(_half(r0), PM // 2), :]), wd_v[:, cols], preferred_element_type=f32)
            acc_s[n, rows, :] = acc + x_v[rows, cols].astype(f32)
        return (11, f)

    def out_proj(r0, m, n):
        rows, cols = pl.ds(r0, m), pl.ds(n * 128, 128)
        acc = lax.dot_general(_upk(o_p[pl.ds(_half(r0), m // 2), :]), _upk(wo_p[pl.ds(n * 64, 64), :]),
                              NT_DIMS, preferred_element_type=f32)
        out_v[rows, cols] = (acc + acc_s[n, rows, :]).astype(bf16)

    def out_copy(r0, m, sem):
        rows = pl.ds(r0, m)
        return pltpu.make_async_copy(out_v.at[rows, :], out_hbm.at[rows, :], sems.at[out_sem0 + sem])

    wait(*w_d, wqkv_cp, wo_cp, wd_cp)
    prep = ([(1, functools.partial(perm_wqkv, t * RP)) for t in range(D // RP)]
            + [(1, functools.partial(perm_wo, t * 128)) for t in range(4)])
    gu = []
    for r in range(S // M1):
        gu += [(min(a + GC, DFM) - a, functools.partial(gate_up, r * M1, M1, a, min(a + GC, DFM)))
               for a in range(G1, DFM, GC)]
        gu += [(DF - DFM, functools.partial(gate_up_tail, r * M1, M1))]
    n_last = len(gu) // (S // M1)
    _interleave(gu[:-n_last], prep)
    for _, f in gu[-n_last:] + qkv_tasks(0):
        f()

    n_tiles = S // PM

    def step(t, last):
        dyn = not isinstance(t, int)
        r = pl.multiple_of(t * PM, PM) if dyn else t * PM
        mxu = [] if last else qkv_tasks(pl.multiple_of(r + PM, PM) if dyn else r + PM)
        mxu += [down_task(r, n) for n in range(4)]
        vpu = [attn_task(r + b * R, dyn and b * R < DIL * WIN) for b in range(PM // R)]
        _interleave(mxu, vpu)
        m = MWL if last else PM
        for i in range(PM // m):
            for n in range(4):
                out_proj(r + i * m, m, n)
            out_copy(r + i * m, m, t + i).start()

    def body(t, carry):
        step(t, False)
        return carry

    lax.fori_loop(0, n_tiles - 1, body, 0)
    step(n_tiles - 1, True)

    for t in range(n_tiles - 1):
        out_copy(t * PM, PM, t).wait()
    for i in range(PM // MWL):
        out_copy((n_tiles - 1) * PM + i * MWL, MWL, n_tiles - 1 + i).wait()


@jax.jit
def pallas_parallel_sum__sliding_local_dilated__glu_gated_geglu__prompt_kernel(
    A_x: jax.Array,
    A_wqkv: jax.Array,
    A_wo: jax.Array,
    B_x: jax.Array,
    B_w_gate: jax.Array,
    B_w_up: jax.Array,
    B_w_down: jax.Array,
):
    del B_x
    hbm = pl.BlockSpec(memory_space=pltpu.HBM)
    out = pl.pallas_call(
        _kernel,
        in_specs=[hbm] * 6,
        out_specs=hbm,
        out_shape=jax.ShapeDtypeStruct((S, D), A_x.dtype),
        scratch_shapes=[
            pltpu.VMEM((S, D), bf16),
            pltpu.VMEM((S // 2, D), i32),
            pltpu.VMEM((DF, D), bf16),
            pltpu.VMEM((DF, D), bf16),
            pltpu.VMEM((DFP, D), bf16),
            pltpu.VMEM((D, 3 * D), bf16),
            pltpu.VMEM((D // 2, 3 * D), i32),
            pltpu.VMEM((D, D), bf16),
            pltpu.VMEM((D // 2, D), i32),
            pltpu.VMEM((S // 2, DFP), i32),
            pltpu.VMEM((4, S, 128), f32),
            pltpu.VMEM((4, S + HALO, 128), f32),
            pltpu.VMEM((4, S + HALO, 128), f32),
            pltpu.VMEM((S // 2, D), i32),
            pltpu.VMEM((S, D), bf16),
            pltpu.VMEM((4, S, 128), f32),
            pltpu.SemaphoreType.DMA((N_SEM,)),
        ],
        compiler_params=pltpu.CompilerParams(
            vmem_limit_bytes=110 * 1024 * 1024,
            flags=FLAGS,
        ),
    )(A_x.reshape(S, D), A_wqkv, A_wo, B_w_gate.T, B_w_up.T, B_w_down)
    return out.reshape(1, S, D)
```
